```python
import jax
import jax.numpy as jnp

def _softmax(x, axis=-1):
    return jax.nn.softmax(x, axis=axis)
def _gelu(x):
    return jax.nn.gelu(x, approximate=True)
def _silu(x):
    return jax.nn.silu(x)
def _sigmoid(x):
    return jax.nn.sigmoid(x)
def _layernorm(x, axis=-1, eps=1e-5):
    m = jnp.mean(x, axis=axis, keepdims=True)
    v = jnp.var(x, axis=axis, keepdims=True)
    return (x - m) / jnp.sqrt(v + eps)
def _scatter_add(tgt, idx, src, axis=0):
    return tgt.at[idx].add(src)
def _segment_sum(src, seg, n):
    return jax.ops.segment_sum(src, seg, n)
class _Rng:
    def __init__(self, key):
        self._k = key
    def _next(self):
        self._k, sub = jax.random.split(self._k)
        return sub
    def normal(self, shape):
        return jax.random.normal(self._next(), shape, dtype=jnp.bfloat16)
    def randint(self, lo, hi, shape):
        return jax.random.randint(self._next(), shape, lo, hi, dtype=jnp.int32)
    def uniform(self, shape, lo=0.0, hi=1.0):
        return jax.random.uniform(self._next(), shape, jnp.bfloat16, lo, hi)
    def permutation(self, n):
        return jax.random.permutation(self._next(), n)


kernel_name = 'recurrent_scan__linear_kernel_hedgehog__dense_activation_relu__prompt'

def _fwd_setup_inputs():
    _rng = _Rng(jax.random.key(int.from_bytes(__import__("os").urandom(4), "little")))
    _w = (lambda a: (lambda t: t.astype(jnp.bfloat16) if jnp.issubdtype(t.dtype, jnp.floating) else t)(jnp.asarray(a)))
    def _A_setup():
        B, S, D, H = 1, 2048, 1024, 32
        Dh = D // H
        return {
            "x": _w((lambda *s: _rng.normal(s) * 0.05)(B, S, D)),
            "wqkv": _w((lambda *s: _rng.normal(s) * 0.05)(D, 3 * D)),
            "w_phi": _w((lambda *s: _rng.normal(s) * 0.05)(H, Dh, Dh) * (Dh ** -0.5)),
            "wo": _w((lambda *s: _rng.normal(s) * 0.05)(D, D)),
        }
    _A_in = _A_setup()

    def _B_setup():
        B, S, D, Dff = 1, 2048, 1024, 3584
        return {
            "x": _w((lambda *s: _rng.normal(s) * 0.05)(B, S, D)),
            "w1": _w((lambda *s: _rng.normal(s) * 0.05)(D, Dff)),
            "w2": _w((lambda *s: _rng.normal(s) * 0.05)(Dff, D)),
        }
    _B_in = _B_setup()

    return {
        "A_x": _A_in["x"],
        "A_wqkv": _A_in["wqkv"],
        "A_w_phi": _A_in["w_phi"],
        "A_wo": _A_in["wo"],
        "B_x": _B_in["x"],
        "B_w1": _B_in["w1"],
        "B_w2": _B_in["w2"],
    }

def _fwd_reference(A_x, A_wqkv, A_w_phi, A_wo, B_x, B_w1, B_w2):
    def _A_ref(x, wqkv, w_phi, wo):
        B, S, D = x.shape
        H = 32; Dh = D // H
        qkv = (lambda x, *d: x.transpose(*d))((x @ wqkv).reshape(B, S, 3, H, Dh), 2, 0, 3, 1, 4)
        q, k, v = qkv[0], qkv[1], qkv[2]
        pq = jnp.einsum("bhsd,hdf->bhsf", q, w_phi)
        pk = jnp.einsum("bhsd,hdf->bhsf", k, w_phi)
        phi_q = jnp.concatenate([_softmax(pq, axis=-1), _softmax(-pq, axis=-1)], axis=-1)
        phi_k = jnp.concatenate([_softmax(pk, axis=-1), _softmax(-pk, axis=-1)], axis=-1)
        kv = jnp.einsum("bhsf,bhsd->bhfd", phi_k, v)
        z  = jnp.einsum("bhsf->bhf", phi_k)
        num = jnp.einsum("bhqf,bhfd->bhqd", phi_q, kv)
        den = jnp.einsum("bhqf,bhf->bhq", phi_q, z)[..., None] + 1e-6
        o = num / den
        return (lambda x, *d: x.transpose(*d))(o, 0, 2, 1, 3).reshape(B, S, D) @ wo

    def _B_ref(x, w1, w2):
        h = jnp.einsum("bsd,df->bsf", x, w1)
        zero = jnp.zeros_like(h)
        h = jnp.maximum(h, zero)
        return jnp.einsum("bsf,fd->bsd", h, w2)

    x = A_x
    xn = _layernorm(x, axis=-1)
    s = _A_ref(xn, A_wqkv, A_w_phi, A_wo)
    g = _silu(_B_ref(xn, B_w1, B_w2))
    return x + s * g


def setup_inputs():
    _inp = _fwd_setup_inputs()
    _gk = jax.random.fold_in(jax.random.key(int.from_bytes(__import__("os").urandom(4), "little")), 2**31 - 1)
    _shapes = [[1, 2048, 1024]]
    _dtypes = ['bfloat16']
    _gks = jax.random.split(_gk, len(_shapes))
    _gs = [jax.random.normal(k, s, dtype=jnp.dtype(d)) * 0.05 for k, s, d in zip(_gks, _shapes, _dtypes)]
    _inp["grad_out"] = _gs[0]
    return _inp

def reference(A_x, A_wqkv, A_w_phi, A_wo, B_w1, B_w2, B_x, grad_out):
    _const = dict(B_x=B_x)
    def _f(*_d):
        return _fwd_reference(**{'A_x': _d[0], 'A_wqkv': _d[1], 'A_w_phi': _d[2], 'A_wo': _d[3], 'B_w1': _d[4], 'B_w2': _d[5], **_const})
    _out, _vjp = jax.vjp(_f, A_x, A_wqkv, A_w_phi, A_wo, B_w1, B_w2)
    _grads = _vjp(grad_out)
    _out0 = jnp.asarray(_out)
    return (_out0, *[jnp.asarray(_g) for _g in _grads])
```

```python
import jax
import jax.numpy as jnp
from jax import lax
import jax.experimental.pallas as pl
import jax.experimental.pallas.tpu as pltpu

F32, BF16, I32 = jnp.float32, jnp.bfloat16, jnp.int32
DH = 32
GW = 128
TS = 512
CF = 512
NN = (((1,), (0,)), ((), ()))
NT = (((1,), (1,)), ((), ()))
TN = (((0,), (0,)), ((), ()))


def _dot(a, b, dims=NN):
    return lax.dot_general(a, b, dims, preferred_element_type=F32)


def _heads(a):
    return a.reshape(a.shape[0] // DH, DH, a.shape[1])


def _dual_softmax(p):
    p3 = _heads(p)
    ep = jnp.exp(p3 - jnp.max(p3, axis=1, keepdims=True))
    em = jnp.exp(jnp.min(p3, axis=1, keepdims=True) - p3)
    ep = ep * (1.0 / jnp.sum(ep, axis=1, keepdims=True))
    em = em * (1.0 / jnp.sum(em, axis=1, keepdims=True))
    return ep.reshape(p.shape), em.reshape(p.shape)


def _dual_softmax_bwd(pp, pm, dp, dm):
    tp, tm = _heads(pp * dp), _heads(pm * dm)
    r = ((tp - tm) - _heads(pp) * jnp.sum(tp, axis=1, keepdims=True)
         + _heads(pm) * jnp.sum(tm, axis=1, keepdims=True))
    return r.reshape(pp.shape)


def _fold_lanes(a):
    r = a[:, 0:128]
    for i in range(1, a.shape[1] // 128):
        r = r + a[:, i * 128:(i + 1) * 128]
    return r


def _tile_lanes(a, n):
    return jnp.concatenate([a] * (n // 128), axis=1)


def _kernel(x_hbm, wqkv_hbm, wphi_ref, wo_hbm, w1_hbm, w2_hbm, go_hbm,
            out_hbm, dx_hbm, dwqkv_hbm, dwphi_ref, dwo_hbm, dw1_hbm, dw2_hbm,
            xn, xnT, rstd, hbuf, php, phm, vT, dqT, df, wq, w1, w2, bd, kv, dkv, zb, dzb,
            dwo_st, in_sem, st_sem):
    S, D = xn.shape
    FF = hbuf.shape[1]
    NTILE, G, NC = S // TS, D // GW, FF // CF
    blk = (lax.broadcasted_iota(I32, (GW, GW), 0) // DH
           == lax.broadcasted_iota(I32, (GW, GW), 1) // DH)
    blk2 = ((lax.broadcasted_iota(I32, (2 * GW, GW), 0) % GW) // DH
            == lax.broadcasted_iota(I32, (2 * GW, GW), 1) // DH)

    def rows(t):
        return pl.ds(pl.multiple_of(t * TS, TS), TS)

    def grp(g):
        return pl.ds(g * GW, GW)

    def forward(xs, gs, wT, wo, tmp, phq, oT, inv, dsb, dwo_acc, ost, sem, osem):
        def x_in(t):
            return pltpu.make_async_copy(x_hbm.at[rows(t)], xs.at[rows(t)], sem.at[t])

        def w_in(i):
            return pltpu.make_async_copy(wqkv_hbm.at[:, pl.ds(i * D, D)], wq.at[:, pl.ds(i * D, D)], in_sem.at[i])
        cp_w1 = pltpu.make_async_copy(w1_hbm, w1, in_sem.at[3])
        cp_w2 = pltpu.make_async_copy(w2_hbm, w2, in_sem.at[4])
        cp_wo = pltpu.make_async_copy(wo_hbm, wo, in_sem.at[5])
        cp_go = pltpu.make_async_copy(go_hbm, gs, in_sem.at[6])
        w_in(1).start()
        x_in(0).start()
        w_in(2).start()
        for t in range(1, NTILE):
            x_in(t).start()
        cp_w1.start()
        w_in(0).start()
        cp_w2.start()
        cp_wo.start()
        cp_go.start()

        sel = (lax.broadcasted_iota(I32, (DH, GW), 0)
               == lax.broadcasted_iota(I32, (DH, GW), 1) % DH).astype(BF16)
        rep = _dot(wphi_ref[...], sel)
        for g in range(G):
            bd[g] = jnp.where(blk, rep[g * GW:(g + 1) * GW], 0.0).astype(BF16)
        kv[...] = jnp.zeros_like(kv)
        dkv[...] = jnp.zeros_like(dkv)
        zb[...] = jnp.zeros_like(zb)
        dzb[...] = jnp.zeros_like(dzb)
        dwo_acc[...] = jnp.zeros_like(dwo_acc)

        def fold_phi(i):
            for g in range(G):
                bdt = bd[g].astype(F32).T.astype(BF16)
                wT[pl.ds(i * D + g * GW, GW), :] = _dot(
                    bdt, wq[:, pl.ds(i * D + g * GW, GW)], NT).astype(BF16)

        w_in(1).wait()
        fold_phi(1)

        def ln(t, c):
            x_in(t).wait()
            x = xs[rows(t), :].astype(F32)
            xc = x - jnp.mean(x, axis=1, keepdims=True)
            r = lax.rsqrt(jnp.mean(xc * xc, axis=1, keepdims=True) + 1e-5)
            y = xc * r
            rstd[rows(t), :] = jnp.broadcast_to(r, (TS, 128))
            xn[rows(t), :] = y.astype(BF16)
            xnT[:, rows(t)] = y.T.astype(BF16)
            return c
        lax.fori_loop(0, NTILE, ln, 0)
        w_in(2).wait()
        for g in range(G):
            wT[pl.ds(2 * D + g * GW, GW), :] = wq[:, pl.ds(2 * D + g * GW, GW)].astype(F32).T.astype(BF16)
        cp_w1.wait()

        def phase1(t, c):
            vT[:, rows(t)] = _dot(wT[pl.ds(2 * D, D), :], xnT[:, rows(t)]).astype(BF16)
            tmp[...] = _dot(wT[pl.ds(D, D), :], xnT[:, rows(t)])
            for g in range(G):
                if g < NC:
                    h = _dot(xn[rows(t), :], w1[:, pl.ds(g * CF, CF)])
                    hb = jnp.where(h > 0, pltpu.bitcast(h, I32), jnp.where(h == 0, 0, -2 ** 31))
                    hbuf[rows(t), pl.ds(g * CF, CF)] = pltpu.bitcast(hb, F32).astype(BF16)
                pp, pm = _dual_softmax(tmp[grp(g), :])
                zb[g, 0:GW] += _fold_lanes(pp)
                zb[g, GW:2 * GW] += _fold_lanes(pm)
                pp, pm = pp.astype(BF16), pm.astype(BF16)
                php[grp(g), rows(t)] = pp
                phm[grp(g), rows(t)] = pm
                kv[g] += _dot(jnp.concatenate([pp, pm], axis=0), vT[grp(g), rows(t)], NT)
            return c
        with jax.named_scope("p1"):
            lax.fori_loop(0, NTILE, phase1, 0)

        for g in range(G):
            kv[g] = jnp.where(blk2, kv[g], 0.0)
            zb[g] = jnp.broadcast_to(jnp.sum(zb[g], axis=1, keepdims=True), (2 * GW, 128))
        w_in(0).wait()
        fold_phi(0)
        cp_w2.wait()
        cp_wo.wait()
        cp_go.wait()

        def o_out(t):
            return pltpu.make_async_copy(ost.at[t % 2], out_hbm.at[rows(t)], osem.at[t % 2])

        def phase2(t, c):
            @pl.when(t >= 2)
            def _():
                o_out(t - 2).wait()
            tmp[...] = _dot(wT[pl.ds(0, D), :], xnT[:, rows(t)])
            fs = []
            for g in range(G):
                fs.append(_dot(hbuf[rows(t), :], w2[:, grp(g)]))
                pp, pm = _dual_softmax(tmp[grp(g), :])
                z = _tile_lanes(zb[g], TS)
                den = jnp.sum(_heads(pp * z[0:GW] + pm * z[GW:2 * GW]), axis=1, keepdims=True) + 1e-6
                iv = jnp.broadcast_to(1.0 / den, (GW // DH, DH, TS)).reshape(GW, TS)
                ph = jnp.concatenate([pp.astype(BF16), pm.astype(BF16)], axis=0)
                phq[g] = ph
                inv[grp(g), :] = iv
                o = _dot(kv[g].T.astype(BF16), ph) * iv
                tmp[grp(g), :] = o
                oT[grp(g), :] = o.astype(BF16)
            s = _dot(tmp[...].T.astype(BF16), wo[...])
            for g in range(G):
                f = fs[g]
                sg = jax.nn.sigmoid(f)
                gate = f * sg
                sv = s[:, g * GW:(g + 1) * GW]
                go = gs[rows(t), grp(g)].astype(F32)
                ost[t % 2, :, grp(g)] = (xs[rows(t), grp(g)].astype(F32) + sv * gate).astype(BF16)
                dsb[:, grp(g)] = (go * gate).astype(BF16)
                df[rows(t), grp(g)] = (go * sv * (sg + gate * (1.0 - sg))).astype(BF16)
            o_out(t).start()
            doT = _dot(wo[...], dsb[...], NT)
            for g in range(G):
                dwo_acc[:, grp(g)] += _dot(oT[...], dsb[:, grp(g)])
                dn = doT[g * GW:(g + 1) * GW] * inv[grp(g), :]
                dd = -jnp.sum(_heads(dn * tmp[grp(g), :]), axis=1, keepdims=True)
                dd = jnp.broadcast_to(dd, (GW // DH, DH, TS)).reshape(GW, TS)
                dn = dn.astype(BF16)
                ph = phq[g]
                dkv[g] += _dot(ph, dn, NT)
                dph = _dot(kv[g].astype(BF16), dn)
                z = _tile_lanes(zb[g], TS)
                pp, pm = ph[0:GW].astype(F32), ph[GW:2 * GW].astype(F32)
                dzb[g, 0:GW] += _fold_lanes(pp * dd)
                dzb[g, GW:2 * GW] += _fold_lanes(pm * dd)
                dqT[grp(g), rows(t)] = _dual_softmax_bwd(
                    pp, pm, dph[0:GW] + z[0:GW] * dd, dph[GW:2 * GW] + z[GW:2 * GW] * dd).astype(BF16)
            return c
        with jax.named_scope("p2"):
            lax.fori_loop(0, NTILE, phase2, 0)
        dwo_st[...] = dwo_acc[...].astype(BF16)
        o_out(NTILE - 2).wait()
        o_out(NTILE - 1).wait()

    pl.run_scoped(
        forward, pltpu.VMEM((S, D), BF16), pltpu.VMEM((S, D), BF16), pltpu.VMEM((3 * D, D), BF16),
        pltpu.VMEM((D, D), BF16), pltpu.VMEM((D, TS), F32), pltpu.VMEM((G, 2 * GW, TS), BF16),
        pltpu.VMEM((D, TS), BF16), pltpu.VMEM((D, TS), F32), pltpu.VMEM((TS, D), BF16),
        pltpu.VMEM((D, D), F32), pltpu.VMEM((2, TS, D), BF16),
        pltpu.SemaphoreType.DMA((NTILE,)), pltpu.SemaphoreType.DMA((2,)))

    cp_dwo = pltpu.make_async_copy(dwo_st, dwo_hbm, st_sem.at[0])
    cp_dwo.start()

    def backward(dxn, dhb, st1, st2, stw, stx, gs, sem1, sem2, semw, semx, semg):
        cp_go = pltpu.make_async_copy(go_hbm, gs, semg.at[0])
        cp_go.start()

        def chunk(c):
            return pl.ds(pl.multiple_of(c * CF, CF), CF)

        def w1_out(c):
            return pltpu.make_async_copy(st1.at[c % 2], dw1_hbm.at[:, chunk(c)], sem1.at[c % 2])

        def w2_out(c):
            return pltpu.make_async_copy(st2.at[c % 2], dw2_hbm.at[chunk(c)], sem2.at[c % 2])

        dxn[...] = jnp.zeros_like(dxn)

        def phase3(c, carry):
            @pl.when(c >= 2)
            def _():
                w1_out(c - 2).wait()
                w2_out(c - 2).wait()
            hc = hbuf[:, chunk(c)]
            st2[c % 2] = _dot(hc, df[...], TN).astype(BF16)
            t = _dot(df[...], w2[chunk(c), :], NT)
            hb = pltpu.bitcast(hc.astype(F32), I32)
            dhb[...] = jnp.where(hb > 0, t, jnp.where(hb == 0, 0.5 * t, 0.0)).astype(BF16)
            st1[c % 2] = _dot(xnT[...], dhb[...]).astype(BF16)
            dxn[...] += _dot(dhb[...], w1[:, chunk(c)], NT)
            w1_out(c).start()
            w2_out(c).start()
            return carry
        with jax.named_scope("p3"):
            lax.fori_loop(0, NC, phase3, 0)

        def gsl(g, i=0):
            return pl.ds(pl.multiple_of(i * D + g * GW, GW), GW)

        def w_out(g, i):
            return pltpu.make_async_copy(stw.at[g % 2, i], dwqkv_hbm.at[:, gsl(g, i)], semw.at[(g % 2) * 3 + i])

        def phase4(g, carry):
            @pl.when(g >= 2)
            def _():
                for i in range(3):
                    w_out(g - 2, i).wait()
            b = bd[g]

            def unfold(i, dwp):
                dwp = dwp.astype(BF16)
                w = wq[:, gsl(g, i)]
                stw[g % 2, i] = _dot(dwp, b, NT).astype(BF16)
                wq[:, gsl(g, i)] = _dot(w, b).astype(BF16)
                return _dot(w, dwp, TN)
            m = unfold(0, _dot(xnT[...], dqT[gsl(g), :], NT))
            dk = jnp.where(blk2, dkv[g], 0.0)
            dz = jnp.sum(dzb[g], axis=1, keepdims=True)
            ph = jnp.concatenate([php[gsl(g), :], phm[gsl(g), :]], axis=0)
            dph = _dot(dk.astype(BF16), vT[gsl(g), :]) + dz
            dv = _dot(dk.T.astype(BF16), ph).astype(BF16)
            vT[gsl(g), :] = dv
            stw[g % 2, 2] = _dot(xnT[...], dv, NT).astype(BF16)
            dk_ = _dual_softmax_bwd(ph[0:GW].astype(F32), ph[GW:2 * GW].astype(F32),
                                    dph[0:GW], dph[GW:2 * GW]).astype(BF16)
            php[gsl(g), :] = dk_
            m = m + unfold(1, _dot(xnT[...], dk_, NT))
            for i in range(GW // DH):
                dwphi_ref[pl.ds(pl.multiple_of(g * GW + i * DH, DH), DH), :] = (
                    m[i * DH:(i + 1) * DH, i * DH:(i + 1) * DH].astype(BF16))
            for i in range(3):
                w_out(g, i).start()
            return carry
        with jax.named_scope("p4"):
            lax.fori_loop(0, G, phase4, 0)
        for c in (NC - 2, NC - 1):
            w1_out(c).wait()
            w2_out(c).wait()
        cp_go.wait()

        def x_out(t):
            return pltpu.make_async_copy(stx.at[t % 2], dx_hbm.at[rows(t)], semx.at[t % 2])

        def phase5(t, carry):
            @pl.when(t >= 2)
            def _():
                x_out(t - 2).wait()
            a = (_dot(wq[:, 0:D], dqT[:, rows(t)]) + _dot(wq[:, D:2 * D], php[:, rows(t)])
                 + _dot(wq[:, 2 * D:3 * D], vT[:, rows(t)]))
            d = a.T + dxn[rows(t), :]
            y = xn[rows(t), :].astype(F32)
            d = d - jnp.mean(d, axis=1, keepdims=True) - y * jnp.mean(d * y, axis=1, keepdims=True)
            stx[t % 2] = (gs[rows(t), :].astype(F32) + d * _tile_lanes(rstd[rows(t), :], D)).astype(BF16)
            x_out(t).start()
            return carry
        with jax.named_scope("p5"):
            lax.fori_loop(0, NTILE, phase5, 0)
        for g in (G - 2, G - 1):
            for i in range(3):
                w_out(g, i).wait()
        x_out(NTILE - 2).wait()
        x_out(NTILE - 1).wait()

    pl.run_scoped(
        backward, pltpu.VMEM((S, D), F32), pltpu.VMEM((S, CF), BF16), pltpu.VMEM((2, D, CF), BF16),
        pltpu.VMEM((2, CF, D), BF16), pltpu.VMEM((2, 3, D, GW), BF16), pltpu.VMEM((2, TS, D), BF16),
        pltpu.VMEM((S, D), BF16), pltpu.SemaphoreType.DMA((2,)), pltpu.SemaphoreType.DMA((2,)),
        pltpu.SemaphoreType.DMA((6,)), pltpu.SemaphoreType.DMA((2,)), pltpu.SemaphoreType.DMA((1,)))
    cp_dwo.wait()


@jax.jit
def pallas_recurrent_scan__linear_kernel_hedgehog__dense_activation_relu__prompt_kernel(
    A_x: jax.Array,
    A_wqkv: jax.Array,
    A_w_phi: jax.Array,
    A_wo: jax.Array,
    B_x: jax.Array,
    B_w1: jax.Array,
    B_w2: jax.Array,
    grad_out: jax.Array,
):
    del B_x
    B, S, D = A_x.shape
    assert B == 1
    FF = B_w1.shape[1]
    G = D // GW
    hbm = pl.BlockSpec(memory_space=pl.ANY)
    vmem = pl.BlockSpec(memory_space=pltpu.VMEM)
    sds = lambda *s: jax.ShapeDtypeStruct(s, BF16)
    out, dx, dwqkv, dwphi, dwo, dw1, dw2 = pl.pallas_call(
        _kernel,
        in_specs=[hbm, hbm, vmem, hbm, hbm, hbm, hbm],
        out_specs=[hbm, hbm, hbm, vmem, hbm, hbm, hbm],
        out_shape=[sds(S, D), sds(S, D), sds(D, 3 * D), sds(D, DH), sds(D, D), sds(D, FF), sds(FF, D)],
        scratch_shapes=[
            pltpu.VMEM((S, D), BF16), pltpu.VMEM((D, S), BF16), pltpu.VMEM((S, 128), F32),
            pltpu.VMEM((S, FF), BF16), pltpu.VMEM((D, S), BF16), pltpu.VMEM((D, S), BF16),
            pltpu.VMEM((D, S), BF16), pltpu.VMEM((D, S), BF16), pltpu.VMEM((S, D), BF16),
            pltpu.VMEM((D, 3 * D), BF16), pltpu.VMEM((D, FF), BF16), pltpu.VMEM((FF, D), BF16),
            pltpu.VMEM((G, GW, GW), BF16), pltpu.VMEM((G, 2 * GW, GW), F32),
            pltpu.VMEM((G, 2 * GW, GW), F32), pltpu.VMEM((G, 2 * GW, 128), F32),
            pltpu.VMEM((G, 2 * GW, 128), F32), pltpu.VMEM((D, D), BF16),
            pltpu.SemaphoreType.DMA((7,)), pltpu.SemaphoreType.DMA((1,)),
        ],
        compiler_params=pltpu.CompilerParams(vmem_limit_bytes=126 * 1024 * 1024),
    )(A_x.reshape(S, D), A_wqkv, A_w_phi.reshape(D, DH), A_wo, B_w1, B_w2, grad_out.reshape(S, D))
    return (out.reshape(B, S, D), dx.reshape(B, S, D), dwqkv, dwphi.reshape(A_w_phi.shape),
            dwo, dw1, dw2)
```

```python
import functools

import jax
import jax.numpy as jnp
from jax import lax
import jax.experimental.pallas as pl
import jax.experimental.pallas.tpu as pltpu

F32, BF16, I32 = jnp.float32, jnp.bfloat16, jnp.int32
DH = 32
GW = 128
TS = 512
PW = 256
CF = 512
HALVES = (slice(0, GW // 2), slice(GW // 2, GW))
SUM_A, SUM_B = (0, 1, 4, 5, 6), (0, 2, 3, 5, 6)
NN = (((1,), (0,)), ((), ()))
NT = (((1,), (1,)), ((), ()))
TN = (((0,), (0,)), ((), ()))


def _dot(a, b, dims=NN):
    return lax.dot_general(a, b, dims, preferred_element_type=F32)


def _heads(a):
    return a.reshape(a.shape[0] // DH, DH, a.shape[1])


def _dual_softmax(p):
    p3 = _heads(p)
    ep = jnp.exp(p3 - jnp.max(p3, axis=1, keepdims=True))
    em = jnp.exp(jnp.min(p3, axis=1, keepdims=True) - p3)
    ep = ep * (1.0 / jnp.sum(ep, axis=1, keepdims=True))
    em = em * (1.0 / jnp.sum(em, axis=1, keepdims=True))
    return ep.reshape(p.shape), em.reshape(p.shape)


def _dual_softmax_bwd(pp, pm, dp, dm):
    tp, tm = _heads(pp * dp), _heads(pm * dm)
    r = ((tp - tm) - _heads(pp) * jnp.sum(tp, axis=1, keepdims=True)
         + _heads(pm) * jnp.sum(tm, axis=1, keepdims=True))
    return r.reshape(pp.shape)


def _fold_lanes(a):
    r = a[:, 0:128]
    for i in range(1, a.shape[1] // 128):
        r = r + a[:, i * 128:(i + 1) * 128]
    return r


def _per_head(a):
    return jnp.concatenate([a[h] for h in range(a.shape[0]) for _ in range(DH // 8)], axis=0)


def _tile_lanes(a, n):
    return jnp.concatenate([a] * (n // 128), axis=1)


def _quads(a):
    r, c = a.shape[0] // 2, a.shape[1] // 2
    return a[:r, :c], a[:r, c:], a[r:, :c], a[r:, c:]


def _bf(*xs):
    return [x.astype(BF16) for x in xs]


def _in_a(a11, a12, a21, a22):
    return _bf(a11 + a22, a21 + a22, a11, a22, a11 + a12, a21 - a11, a12 - a22)


def _in_b(b11, b12, b21, b22):
    return _bf(b11 + b22, b11, b12 - b22, b21 - b11, b22, b11 + b12, b21 + b22)


def _in_c(g11, g12, g21, g22):
    return _bf(g11 + g22, g21 - g22, g12 + g22, g11 + g21, g12 - g11, g22, g11)


def _out_a(m):
    return m[0] + m[2] + m[4] - m[5], m[4] + m[6], m[1] + m[5], m[0] + m[1] + m[3] - m[6]


def _out_b(m):
    return m[0] + m[1] - m[3] + m[5], m[2] + m[5], m[3] + m[6], m[0] - m[2] + m[4] + m[6]


def _out_c(m):
    return m[0] + m[3] - m[4] + m[6], m[2] + m[4], m[1] + m[3], m[0] - m[1] + m[2] + m[5]


class _Packed:
    def __init__(self, ref):
        self.ref = ref
        self.shape = ref.shape[:-2] + (2 * ref.shape[-2], ref.shape[-1])

    def _index(self, idx):
        idx = () if idx is Ellipsis else idx if isinstance(idx, tuple) else (idx,)
        idx = list(idx) + [slice(None)] * (len(self.shape) - len(idx))
        r = idx[-2]
        if isinstance(r, slice):
            lo, hi, _ = r.indices(self.shape[-2])
            r = pl.ds(lo, hi - lo)
        start = r.start // 2 if isinstance(r.start, int) else pl.multiple_of(lax.shift_right_logical(r.start, 1), 8)
        idx[-2] = pl.ds(start, r.size // 2)
        return tuple(idx)

    def __getitem__(self, idx):
        return pltpu.bitcast(self.ref[self._index(idx)], BF16)

    def __setitem__(self, idx, val):
        self.ref[self._index(idx)] = pltpu.bitcast(val, I32)


def _pk(*shape):
    return pltpu.VMEM(shape[:-2] + (shape[-2] // 2, shape[-1]), I32)


def _by_pair(pp, pm):
    return [jnp.concatenate([pp[h], pm[h]], axis=0) for h in HALVES]


def _state(a, ph):
    return jnp.concatenate([_dot(a[h], p, NT) for h, p in zip(HALVES, ph)], axis=0)


def _apply(st, ph):
    return jnp.concatenate([_dot(st[h], p) for h, p in zip(HALVES, ph)], axis=0)


def _own_head(st):
    r = lax.broadcasted_iota(I32, (GW, GW), 0)
    c = lax.broadcasted_iota(I32, (GW, GW), 1)
    st = jnp.where((r // DH) % 2 == (c // DH) % 2, st, 0.0)
    t = st.T
    t = jnp.concatenate([t[HALVES[0]], t[HALVES[0]], t[HALVES[1]], t[HALVES[1]]], axis=0)
    r = lax.broadcasted_iota(I32, (2 * GW, GW), 0)
    c = lax.broadcasted_iota(I32, (2 * GW, GW), 1)
    return st.astype(BF16), jnp.where((r % GW) // DH == c // DH, t, 0.0).astype(BF16)


def _kernel(x_hbm, wqkv_hbm, wphi_ref, wo_hbm, w1_hbm, w2_hbm, go_hbm,
            out_hbm, dx_hbm, dwqkv_hbm, dwphi_ref, dwo_hbm, dw1_hbm, dw2_hbm,
            xn, rstd, hbuf, php, phm, vT, dqT, gdf, gdfT, axT, wq, wf, w1, w2, bd, dkv, dzb,
            dwo_acc, xs, in_sem, st_sem, osem):
    xn, hbuf, php, phm, vT, dqT, gdf, gdfT, axT, wf, bd = map(
        _Packed, (xn, hbuf, php, phm, vT, dqT, gdf, gdfT, axT, wf, bd))
    S, D = xn.shape
    FF = hbuf.shape[1]
    NTILE, G, NC, NP = S // TS, D // GW, FF // CF, D // PW
    blk = (lax.broadcasted_iota(I32, (GW, GW), 0) // DH
           == lax.broadcasted_iota(I32, (GW, GW), 1) // DH)
    assert NP == NTILE and FF >= 7 * D // 2

    def rows(t):
        return pl.ds(pl.multiple_of(t * TS, TS), TS)

    def half(t):
        return pl.ds(pl.multiple_of(t * (TS // 2), TS // 2), TS // 2)

    def gsl(g, i=0):
        return pl.ds(pl.multiple_of(i * D + g * GW, GW), GW)

    def pair(p, i=0):
        return pl.ds(pl.multiple_of(i * D + p * PW, PW), PW)

    def o_out(t):
        return pltpu.make_async_copy(xs.at[rows(t)], out_hbm.at[rows(t)], osem.at[t])

    def forward(kv, zb, gs, wT, wo, zacc, fbuf, kvt, kvn, phq, o32, oT, onat, inv, gate_s, gd_s, dsb,
                sem, wsem):
        wT, kvt, kvn, phq, oT, onat, dsb = map(_Packed, (wT, kvt, kvn, phq, oT, onat, dsb))
        HC = FF // NP

        def hcols(p):
            return pl.ds(pl.multiple_of(p * HC, 128), HC)

        def x_in(t):
            return pltpu.make_async_copy(x_hbm.at[rows(t)], xs.at[rows(t)], sem.at[t])

        def w_in(p, i):
            if i == 3:
                return pltpu.make_async_copy(w1_hbm.at[:, hcols(p)], w1.at[:, hcols(p)], wsem.at[i])
            return pltpu.make_async_copy(wqkv_hbm.at[:, pair(p, i)], wq.at[:, pair(p, i)], wsem.at[i])
        cp_w2 = pltpu.make_async_copy(w2_hbm, w2, in_sem.at[0])
        cp_wo = pltpu.make_async_copy(wo_hbm, wo, in_sem.at[1])
        cp_go = pltpu.make_async_copy(go_hbm, gs, in_sem.at[2])
        for j in range(3):
            w_in(0, j).start()
        x_in(0).start()
        w_in(0, 3).start()

        sel = (lax.broadcasted_iota(I32, (DH, GW), 0)
               == lax.broadcasted_iota(I32, (DH, GW), 1) % DH).astype(BF16)

        def init(g, c):
            bd[g] = jnp.where(blk, _dot(wphi_ref[gsl(g), :], sel), 0.0).astype(BF16)
            for r in (kv, dkv, zacc, dzb):
                r[g] = jnp.zeros(r.shape[1:], F32)
            dwo_acc[gsl(g), :] = jnp.zeros((GW, D), F32)
            return c
        lax.fori_loop(0, G, init, 0)
        fbuf[...] = jnp.zeros_like(fbuf)

        def phase1(p, c):
            for j in range(3):
                w_in(p, j).wait()

            for n in range(3):
                w = [wq[:, gsl(2 * p + j, n)] for j in range(2)]
                if n < 2:
                    w = [_dot(w[j], bd[2 * p + j]) for j in range(2)]
                    for j in range(2):
                        wf[:, gsl(2 * p + j, n)] = w[j].astype(BF16)
                for u in range(NP):
                    quads = [b[(2 * u + a) * GW:(2 * u + a + 1) * GW].astype(F32) for a in range(2) for b in w]
                    for i, b in enumerate(_in_b(*quads)):
                        wT[i, gsl(n), gsl(u)] = b.T

            def tile(t, c):
                @pl.when(p == 0)
                def _():
                    x_in(t).wait()

                    @pl.when(t + 1 < NTILE)
                    def _():
                        x_in(t + 1).start()

                    def norm(k):
                        ys = []
                        for a in range(2):
                            rs = pl.ds(pl.multiple_of(t * TS + a * (TS // 2) + k, 16), 16)
                            x = xs[rs, :].astype(F32)
                            xc = x - jnp.mean(x, axis=1, keepdims=True)
                            r = lax.rsqrt(jnp.mean(xc * xc, axis=1, keepdims=True) + 1e-5)
                            rstd[rs, :] = jnp.broadcast_to(r, (16, 128))
                            ys.append(xc * r)
                            xn[rs, :] = ys[a].astype(BF16)
                        quads = [jnp.concatenate([y[:, (2 * u + b) * GW:(2 * u + b + 1) * GW] for u in range(NP)], axis=1)
                                 for y in ys for b in range(2)]
                        for i, a in enumerate(_in_a(*quads)):
                            gdf[i, pl.ds(pl.multiple_of(t * (TS // 2) + k, 16), 16), :] = a
                    for k in range(0, TS // 2, 16):
                        norm(k)

                def hsl(lo, n):
                    return pl.ds(pl.multiple_of(p * HC + lo, 128), n)

                @pl.when(t == 0)
                def _():
                    w_in(p, 3).wait()

                    @pl.when(p + 1 < NP)
                    def _():
                        for j in range(4):
                            w_in(p + 1, j).start()

                    @pl.when(p == 1)
                    def _():
                        cp_w2.start()

                    @pl.when(p == 2)
                    def _():
                        cp_wo.start()
                        cp_go.start()
                for i in range(7):
                    axT[i, gsl(p), half(t)] = gdf[i, half(t), gsl(p)].T
                e0, o0, e1, o1 = _out_c([_dot(wT[i], gdf[i, half(t), :], NT) for i in range(7)])
                qkv = jnp.concatenate([e0, e1], axis=1), jnp.concatenate([o0, o1], axis=1)

                def relu(h):
                    hb = jnp.where(h > 0, pltpu.bitcast(h, I32), jnp.where(h == 0, 0, -2 ** 31))
                    return pltpu.bitcast(hb, F32).astype(BF16)
                hbuf[rows(t), hsl(0, HC - PW)] = relu(_dot(xn[rows(t), :], w1[:, hsl(0, HC - PW)]))
                for j in range(2):
                    g = p * 2 + j
                    dqT[gsl(g), rows(t)], phq[gsl(g), rows(t)] = _bf(*_dual_softmax(qkv[j][0:GW]))
                    v = qkv[j][2 * GW:3 * GW].astype(BF16)
                    vT[gsl(g), rows(t)] = v
                    pp, pm = _dual_softmax(qkv[j][GW:2 * GW])
                    zs = zacc[g] + jnp.concatenate([_fold_lanes(pp), _fold_lanes(pm)], axis=0)
                    zacc[g] = zs
                    zb[g] = jnp.broadcast_to(jnp.sum(zs, axis=1, keepdims=True), zs.shape)
                    pp, pm = pp.astype(BF16), pm.astype(BF16)
                    php[gsl(g), rows(t)] = pp
                    phm[gsl(g), rows(t)] = pm
                    st = kv[g] + _state(v, _by_pair(pp, pm))
                    kv[g] = st
                    kvt[g], kvn[g] = _own_head(st)
                rest = hsl(HC - PW, PW)
                hbuf[rows(t), rest] = relu(_dot(xn[rows(t), :], w1[:, rest]))
                return c
            lax.fori_loop(0, NTILE, tile, 0)
            return c
        lax.fori_loop(0, NP, phase1, 0)

        cp_w2.wait()
        cp_wo.wait()
        cp_go.wait()

        def phase2(t, c):
            def gating(p):
                f = fbuf[...]
                sg = jax.nn.sigmoid(f)
                gate = f * sg
                go = gs[rows(t), pair(p)].astype(F32)
                gate_s[:, pair(p)] = gate
                gd_s[:, pair(p)] = go * (sg + gate * (1.0 - sg))
                dsb[:, pair(p)] = (go * gate).astype(BF16)

            def fwd_pair(p, c):
                gating(jnp.maximum(p - 1, 0))
                for j in range(2):
                    g = p * 2 + j
                    pp, pm = dqT[gsl(g), rows(t)], phq[gsl(g), rows(t)]
                    z = _tile_lanes(zb[g], TS)
                    den = jnp.sum(_heads(pp.astype(F32) * z[0:GW] + pm.astype(F32) * z[GW:2 * GW]),
                                  axis=1, keepdims=True) + 1e-6
                    iv = jnp.broadcast_to(1.0 / den, (GW // DH, 8, TS))
                    inv[g] = iv
                    o = _apply(kvt[g], _by_pair(pp, pm)) * _per_head(iv)
                    o32[gsl(g), :] = o
                    oT[gsl(g), :] = o.astype(BF16)
                    onat[:, gsl(g)] = o.astype(BF16).T
                fbuf[...] = _dot(hbuf[rows(t), :], w2[:, pair(p)])
                return c
            lax.fori_loop(0, NP, fwd_pair, 0)
            gating(NP - 1)

            def bwd_pair(p, c):
                doT = _dot(wo[pair(p), :], dsb[...], NT)
                sv = _dot(onat[...], wo[:, pair(p)])
                xs[rows(t), pair(p)] = (xs[rows(t), pair(p)].astype(F32)
                                          + sv * gate_s[:, pair(p)]).astype(BF16)
                for i, a in enumerate(_in_c(*_quads(sv * gd_s[:, pair(p)]))):
                    gdf[i, half(t), gsl(p)] = a
                    gdfT[i, gsl(p), half(t)] = a.T
                for j in range(2):
                    g = p * 2 + j
                    dn = doT[j * GW:(j + 1) * GW] * _per_head(inv[g])
                    dd = -jnp.sum(_heads(dn * o32[gsl(g), :]), axis=1, keepdims=True)
                    dd = jnp.broadcast_to(dd, (GW // DH, DH, TS)).reshape(GW, TS)
                    dn = dn.astype(BF16)
                    pp, pm = dqT[gsl(g), rows(t)], phq[gsl(g), rows(t)]
                    dph = _dot(kvn[g], dn)
                    dkv[g] += _state(dn, _by_pair(pp, pm))
                    dwo_acc[:, gsl(g)] += _dot(oT[...], dsb[:, gsl(g)])
                    z = _tile_lanes(zb[g], TS)
                    pp, pm = pp.astype(F32), pm.astype(F32)
                    dzb[g, 0:GW] += _fold_lanes(pp * dd)
                    dzb[g, GW:2 * GW] += _fold_lanes(pm * dd)
                    dqT[gsl(g), rows(t)] = _dual_softmax_bwd(
                        pp, pm, dph[0:GW] + z[0:GW] * dd, dph[GW:2 * GW] + z[GW:2 * GW] * dd).astype(BF16)
                return c
            lax.fori_loop(0, NP, bwd_pair, 0, unroll=2)
            o_out(t).start()
            return c
        lax.fori_loop(0, NTILE, phase2, 0)

    V = pltpu.VMEM
    pl.run_scoped(
        forward, V((G, GW, GW), F32), V((G, 2 * GW, 128), F32), V((S, D), BF16),
        _pk(7, 3 * GW, D // 2), V((D, D), BF16),
        V((G, 2 * GW, 128), F32), V((TS, PW), F32), _pk(G, GW, GW), _pk(G, 2 * GW, GW),
        _pk(D, S), V((D, TS), F32), _pk(D, TS), _pk(TS, D),
        V((G, GW // DH, 8, TS), F32), V((TS, D), F32), V((TS, D), F32), _pk(TS, D),
        pltpu.SemaphoreType.DMA((NTILE,)), pltpu.SemaphoreType.DMA((4,)))

    def backward(gdh, ops, st1, st2, stw, stv, sem1, sem2, semw, semv, semx, semg):
        gdh = _Packed(gdh)
        ops = _Packed(ops)
        cp_go = pltpu.make_async_copy(go_hbm, xs, semg.at[0])

        def chunk(c):
            return pl.ds(pl.multiple_of(c * CF, CF), CF)

        def w1_out(c):
            return pltpu.make_async_copy(st1.at[c % 2], dw1_hbm.at[:, chunk(c)], sem1.at[c % 2])

        def w2_out(c):
            return pltpu.make_async_copy(st2.at[c % 2], dw2_hbm.at[chunk(c)], sem2.at[c % 2])

        def forms(c, p):
            def job(src, r0, c0, nr, nc, fn, keep, slab, dr, dc, s):
                def ld(a, b):
                    return src[pl.ds(pl.multiple_of(r0 + a * nr + s, 16), 16),
                               pl.ds(pl.multiple_of(c0 + b * nc, 128), nc)]
                raw = [ld(0, 0), ld(0, 1), ld(1, 0), ld(1, 1)]
                v = fn(*[a.astype(F32) for a in raw])
                for k, i in enumerate(keep):
                    ops[slab + k + jnp.minimum(p, 0), pl.ds(pl.multiple_of(dr + s, 16), 16),
                        pl.ds(pl.multiple_of(dc, 128), nc)] = v[i]
            hc, ht = CF // 2, TS // 2
            specs = [(w1, p * PW, c * CF, GW, hc, _in_b, SUM_B, 12, p * GW, 0),
                     (w2, c * CF, p * PW, hc, GW, _in_b, SUM_B, 12, D // 2 + p // 2 * hc, p % 2 * GW),
                     (hbuf, p * TS, c * CF, ht, hc, _in_a, SUM_A, 7, p * ht, 0)]
            return [functools.partial(job, *sp, s) for sp in specs for s in range(0, sp[3], 16)]

        def first(p, carry):
            for job in forms(0, p):
                job()
            return carry
        lax.fori_loop(0, NP, first, 0)

        def phase3(c, carry):
            @pl.when(c >= 2)
            def _():
                w1_out(c - 2).wait()
                w2_out(c - 2).wait()

            def act(t, carry):
                def hcol(b):
                    return pl.ds(pl.multiple_of(c * CF + b * (CF // 2), CF // 2), CF // 2)

                def w1_form(i):
                    if i in SUM_B:
                        return ops[12 + SUM_B.index(i), 0:D // 2, :]
                    return jnp.concatenate([w1[gsl(2 * p + i // 4), hcol(i // 4)] for p in range(NP)], axis=0)

                def w2_form(i):
                    if i in SUM_B:
                        a = ops[12 + SUM_B.index(i), D // 2:D // 2 + CF, :]
                        return jnp.concatenate([a[:CF // 2], a[CF // 2:]], axis=1)
                    return jnp.concatenate([w2[hcol(i // 4), gsl(2 * p + i // 4)] for p in range(NP)], axis=1)

                def dw2_part(i):
                    if i in SUM_A:
                        a = ops[7 + SUM_A.index(i), :, gsl(t)]
                    else:
                        a = jnp.concatenate([hbuf[half(2 * u + i - 2), gsl(4 * c + 2 * (i - 2) + t)]
                                             for u in range(NTILE)], axis=0)
                    return _dot(gdfT[i], a)
                da = _out_a([_dot(gdf[i, rows(t), :], w2_form(i), NT) for i in range(7)])
                m, strips = {}, []
                m[2] = dw2_part(2)
                for s, i in enumerate((5, 6, 0, 1)):
                    hb = [pltpu.bitcast(hbuf[gsl(8 * t + s // 2 * 4 + q // 2 * 2 + s % 2), hcol(q % 2)].astype(F32), I32)
                          for q in range(4)]
                    strips.append(_in_c(*[
                        jnp.where(b > 0, a, jnp.where(b == 0, 0.5 * a, 0.0))
                        for a, b in zip([a[s * GW:(s + 1) * GW] for a in da], hb)]))
                    for k in range(7):
                        gdh[k, gsl(4 * t + s), :] = strips[s][k]
                    m[i] = dw2_part(i)

                def dq(i):
                    return _dot(gdh[i, rows(t), :], w1_form(i), NT)

                def add_dxn(q, a):
                    for u in range(2):
                        at = (17 + 4 * q + 2 * t + u,)
                        old = pltpu.bitcast(jnp.where(c > 0, ops.ref[at], 0), F32)
                        ops.ref[at] = pltpu.bitcast(old + a[:, u * PW:(u + 1) * PW], I32)
                q4, q6 = dq(4), dq(6)
                q5 = dq(5)
                add_dxn(1, q4 + q6)
                q1, q0 = dq(1), dq(0)
                add_dxn(2, q1 + q5)
                q2, q3 = dq(2), dq(3)
                add_dxn(0, q0 + q4 - q5 + q2)

                def keep_dw2(q, a):
                    ops[33 + t, rows(q // 2), gsl(q % 2)] = a.astype(BF16)
                m[3] = dw2_part(3)
                add_dxn(3, q0 + q1 - q6 + q3)
                keep_dw2(1, m[2] + m[5])
                m[4] = dw2_part(4)
                keep_dw2(0, m[0] + m[1] + m[5] - m[3])
                keep_dw2(2, m[3] + m[6])
                keep_dw2(3, m[0] - m[2] + m[6] + m[4])
                return carry
            lax.fori_loop(0, NTILE // 2, act, 0)

            def wgt(j, carry):
                nxt = jnp.minimum(c + 1, NC - 1)
                jobs = forms(nxt, 2 * j) + forms(nxt, 2 * j + 1)
                for b in range(2):
                    m = []
                    for i in range(7):
                        n = 7 * b + i
                        m.append(_dot(axT[i, pair(j), :], gdh[i, :, gsl(b)]))
                        for e in range(2) if n < 8 else ():
                            st2[c % 2, gsl(n // 4 * 2 + j), gsl(n % 4 * 2 + e)] = ops[33 + j, gsl(n), gsl(e)].T
                        if n < 13:
                            for job in jobs[n::13]:
                                job()
                            gdh[7 + jnp.minimum(j, 0), 0:16, 0:GW] = ops[33 + j, 0:16, 0:GW]
                    for q, a in enumerate(_out_b(m)):
                        for u in range(2):
                            st1[c % 2, gsl(4 * j + 2 * u + q // 2), gsl(q % 2 * 2 + b)] = (
                                a[u * GW:(u + 1) * GW].astype(BF16))
                return carry
            lax.fori_loop(0, NP // 2, wgt, 0)
            w1_out(c).start()
            w2_out(c).start()
            return carry
        lax.fori_loop(0, NC, phase3, 0)
        for t in range(NTILE):
            o_out(t).wait()
        cp_go.start()

        ht, hd = TS // 2, D // 2

        def w_out(p, i):
            return pltpu.make_async_copy(stw.at[p % 2, i], dwqkv_hbm.at[:, pair(p, i)], semw.at[(p % 2) * 2 + i])

        def interleave(top, bot):
            return jnp.concatenate(
                [v[u * GW:(u + 1) * GW] for u in range(top.shape[0] // GW) for v in (top, bot)], axis=0)

        def weight_forms(src, c1, c2, store, part):
            for u in range(2 * part, 2 * part + 2):
                for s in range(0, GW, 32):
                    v = _in_b(*[src[pl.ds((2 * u + a) * GW + s, 32), cs].astype(F32)
                                for a in range(2) for cs in (c1, c2)])
                    for i in range(7):
                        store(i, u * GW + s, v[i])

        def phase4(p, carry):
            @pl.when(p >= 2)
            def _():
                for i in range(2):
                    w_out(p - 2, i).wait()
            dws = []
            state = [_own_head(dkv[2 * p + j]) for j in range(2)]

            dz = [jnp.sum(dzb[2 * p + j], axis=1, keepdims=True) for j in range(2)]

            def keep(n, u, s, e, o):
                for i, a in enumerate(_in_c(e[:, :ht], o[:, :ht], e[:, ht:], o[:, ht:])):
                    gdh[i, pl.ds((n * NTILE + u) * GW + s, DH), :] = a

            def queries():
                for u in range(NTILE):
                    for s in range(0, GW, DH):
                        keep(0, u, s, *[dqT[pl.ds(pl.multiple_of((2 * p + j) * GW + s, DH), DH),
                                            pl.ds(u * TS, TS)].astype(F32) for j in range(2)])

            def keys(u):
                ts, dk = pl.ds(u * TS, TS), []
                for j in range(2):
                    g = 2 * p + j
                    dph = _dot(state[j][1], vT[gsl(g), ts]) + dz[j]
                    dk.append(_dual_softmax_bwd(php[gsl(g), ts].astype(F32), phm[gsl(g), ts].astype(F32),
                                                dph[0:GW], dph[GW:2 * GW]))
                for s in range(0, GW, DH):
                    keep(1, u, s, dk[0][s:s + DH], dk[1][s:s + DH])

            def values():
                for u in range(NTILE):
                    ts = pl.ds(u * TS, TS)
                    dv = [_apply(state[j][0], _by_pair(php[gsl(2 * p + j), ts], phm[gsl(2 * p + j), ts]))
                          for j in range(2)]
                    for i, a in enumerate(_in_c(dv[0][:, :ht], dv[1][:, :ht], dv[0][:, ht:], dv[1][:, ht:])):
                        gdfT[i, gsl(p), pl.ds(u * ht, ht)] = a

            def weights(n, after):
                j, dst = n // 2, (gdf, gdf, ops)[n // 2]
                spare = (7 + jnp.minimum(p, 0), slice(0, 16), slice(0, GW))

                def store(i, r, v):
                    dst[i, pl.ds(pl.multiple_of(p // 2 * hd + r, 32), 32), gsl(p % 2 * 2 + j if j < 2 else p % 2)] = v
                if n % 2 == 0:
                    dst[spare] = after[0:16].astype(BF16)
                if j < 2:
                    weight_forms(wf, gsl(2 * p, j), gsl(2 * p + 1, j), store, n % 2)
                else:
                    weight_forms(wq, gsl(2 * p, 2), gsl(2 * p + 1, 2), store, n % 2)
                if n % 2 == 1:
                    gdh[spare] = dst[spare]

            def products(j):
                m = []
                for i in range(7):
                    a = jnp.concatenate([gdh[i, pl.ds((j * NTILE + u) * GW, GW), :] for u in range(NTILE)], axis=1)
                    m.append(_dot(axT[i], a, NT))
                    for b in range(2):
                        hbuf[gsl(b * G + 2 * p + j), pl.ds(i * hd, hd)] = a[:, b * hd:(b + 1) * hd]
                    if j == 0 and i < NTILE:
                        keys(i)
                    if j == 1 and i < 6:
                        weights(i, dws[0][i % 4] if i == 0 else m[i - 1])
                dws.append(_bf(*_out_b(m)))

            def unfold(i, j):
                dwp = interleave(dws[i][j], dws[i][2 + j])
                stw[p % 2, i, :, pl.ds(j * GW, GW)] = _dot(dwp, bd[2 * p + j], NT).astype(BF16)
                return _dot(wq[:, gsl(2 * p + j, i)], dwp, TN)
            values()
            queries()
            products(0)
            products(1)
            mq = [unfold(0, j) for j in range(2)]
            for j in range(2):
                m = mq[j] + unfold(1, j)
                for i in range(GW // DH):
                    dwphi_ref[pl.ds(pl.multiple_of((2 * p + j) * GW + i * DH, DH), DH), :] = (
                        m[i * DH:(i + 1) * DH, i * DH:(i + 1) * DH].astype(BF16))
            for i in range(2):
                w_out(p, i).start()
            return carry
        lax.fori_loop(0, NP, phase4, 0)
        for c in (NC - 2, NC - 1):
            w1_out(c).wait()
            w2_out(c).wait()
        cp_go.wait()

        def wo_out(t):
            return pltpu.make_async_copy(st2.at[t // 4, gsl(t % 4)], dwo_hbm.at[gsl(t)], st_sem.at[t % 2])

        def tok(t, a):
            return gsl(t // 2 * 4 + a * 2 + t % 2)

        def x_out(t, a):
            return pltpu.make_async_copy(xs.at[tok(t, a)], dx_hbm.at[tok(t, a)], semx.at[t % 2 * 2 + a])

        def v_out(t):
            r = pl.ds(pl.multiple_of(t % 2 * hd, hd), hd)
            return pltpu.make_async_copy(stv.at[t % 2], dwqkv_hbm.at[r, pair(t // 2, 2)], semv.at[t % 2])

        def phase5(t, carry):
            @pl.when(t >= 2)
            def _():
                v_out(t - 2).wait()
                wo_out(t - 2).wait()
                for a in range(2):
                    x_out(t - 2, a).wait()

            def part(i):
                w = jnp.concatenate([gdf[i, 0:hd, :], gdf[i, hd:D, :], ops[i, 0:hd, :], ops[i, hd:D, :]], axis=1)
                d = jnp.concatenate([hbuf[pl.ds(pl.multiple_of(t // 4 * D, D), D), gsl(4 * i + t % 4)],
                                     gdfT[i, :, gsl(t)]], axis=0)
                return _dot(w, d)
            st2[t // 4, gsl(t % 4), :] = dwo_acc[gsl(t), :].astype(BF16)
            da = _out_a([part(i) for i in range(7)])
            m = []

            def dwv_part():
                m.append(_dot(axT[len(m), pair(t % 2), :], gdfT[len(m), gsl(t // 2), :], NT))

            def slot(a, s):
                return (7 + jnp.minimum(t, 0), pl.ds(pl.multiple_of((a + t) % 2 * GW + s, 64), 64))
            dwv_part()
            for a in range(2):
                d = interleave(da[2 * a], da[2 * a + 1]).T + pltpu.bitcast(jnp.concatenate(
                    [ops.ref[17 + 4 * (2 * a + b) + t // 4 * 2 + u // 2, gsl(t % 4), pl.ds(u % 2 * GW, GW)]
                     for u in range(NP) for b in range(2)], axis=1), F32)
                for s in (0, 64):
                    gdfT.ref[slot(a, s)] = pltpu.bitcast(d[s:s + 64], I32)
                dwv_part()
            for a in range(2):
                for s in (0, 64):
                    r = pl.ds(pl.multiple_of(tok(t, a).start + s, 64), 64)
                    d = pltpu.bitcast(gdfT.ref[slot(a, s)], F32)
                    y = xn[r, :].astype(F32)
                    d = d - jnp.mean(d, axis=1, keepdims=True) - y * jnp.mean(d * y, axis=1, keepdims=True)
                    d = xs[r, :].astype(F32) + d * _tile_lanes(rstd[r, :], D)
                    xs[r, :] = d.astype(BF16)
                    gdfT.ref[slot(a, s) + (pl.ds(0, GW),)] = pltpu.bitcast(d[:, D - GW:], I32)
                    dwv_part()
            d11, d12, d21, d22 = _bf(*_out_b(m))
            stv[t % 2, :, 0:GW] = interleave(d11, d21)
            stv[t % 2, :, GW:PW] = interleave(d12, d22)
            v_out(t).start()
            wo_out(t).start()
            for a in range(2):
                x_out(t, a).start()
            return carry
        lax.fori_loop(0, 2 * NTILE, phase5, 0)
        for p in (NP - 2, NP - 1):
            for i in range(2):
                w_out(p, i).wait()
        for t in (2 * NTILE - 2, 2 * NTILE - 1):
            v_out(t).wait()
            wo_out(t).wait()
            for a in range(2):
                x_out(t, a).wait()

    pl.run_scoped(
        backward, _pk(8, S // 2, CF // 2), _pk(35, S // 2, CF // 2), pltpu.VMEM((2, D, CF), BF16),
        pltpu.VMEM((2, CF, D), BF16), V((2, 2, D, PW), BF16), V((2, D // 2, PW), BF16),
        pltpu.SemaphoreType.DMA((2,)), pltpu.SemaphoreType.DMA((2,)),
        pltpu.SemaphoreType.DMA((4,)), pltpu.SemaphoreType.DMA((2,)), pltpu.SemaphoreType.DMA((4,)),
        pltpu.SemaphoreType.DMA((1,)))


@jax.jit
def pallas_recurrent_scan__linear_kernel_hedgehog__dense_activation_relu__prompt_kernel(
    A_x: jax.Array,
    A_wqkv: jax.Array,
    A_w_phi: jax.Array,
    A_wo: jax.Array,
    B_x: jax.Array,
    B_w1: jax.Array,
    B_w2: jax.Array,
    grad_out: jax.Array,
):
    del B_x
    B, S, D = A_x.shape
    assert B == 1
    FF = B_w1.shape[1]
    G = D // GW
    hbm = pl.BlockSpec(memory_space=pl.ANY)
    vmem = pl.BlockSpec(memory_space=pltpu.VMEM)
    sds = lambda *s: jax.ShapeDtypeStruct(s, BF16)
    out, dx, dwqkv, dwphi, dwo, dw1, dw2 = pl.pallas_call(
        _kernel,
        in_specs=[hbm, hbm, vmem, hbm, hbm, hbm, hbm],
        out_specs=[hbm, hbm, hbm, vmem, hbm, hbm, hbm],
        out_shape=[sds(S, D), sds(S, D), sds(D, 3 * D), sds(D, DH), sds(D, D), sds(D, FF), sds(FF, D)],
        scratch_shapes=[
            _pk(S, D), pltpu.VMEM((S, 128), F32), _pk(S, FF),
            _pk(D, S), _pk(D, S), _pk(D, S), _pk(D, S), _pk(8, S // 2, D // 2),
            _pk(8, D // 2, S // 2), _pk(7, D // 2, S // 2),
            pltpu.VMEM((D, 3 * D), BF16), _pk(D, 2 * D), pltpu.VMEM((D, FF), BF16),
            pltpu.VMEM((FF, D), BF16), _pk(G, GW, GW), pltpu.VMEM((G, GW, GW), F32),
            pltpu.VMEM((G, 2 * GW, 128), F32), pltpu.VMEM((D, D), F32), pltpu.VMEM((S, D), BF16),
            pltpu.SemaphoreType.DMA((3,)), pltpu.SemaphoreType.DMA((2,)),
            pltpu.SemaphoreType.DMA((S // TS,)),
        ],
        compiler_params=pltpu.CompilerParams(vmem_limit_bytes=127 * 1024 * 1024),
    )(A_x.reshape(S, D), A_wqkv, A_w_phi.reshape(D, DH), A_wo, B_w1, B_w2, grad_out.reshape(S, D))
    return (out.reshape(B, S, D), dx.reshape(B, S, D), dwqkv, dwphi.reshape(A_w_phi.shape),
            dwo, dw1, dw2)
```
